```python
import os as _os
_os.environ.setdefault("JAX_PLATFORMS", "cpu")
import jax
import jax.numpy as jnp

def _softmax(x, axis=-1):
    return jax.nn.softmax(x, axis=axis)
def _gelu(x):
    return jax.nn.gelu(x, approximate=True)
def _silu(x):
    return jax.nn.silu(x)
def _sigmoid(x):
    return jax.nn.sigmoid(x)
def _layernorm(x, axis=-1, eps=1e-5):
    m = jnp.mean(x, axis=axis, keepdims=True)
    v = jnp.var(x, axis=axis, keepdims=True)
    return (x - m) / jnp.sqrt(v + eps)
def _scatter_add(tgt, idx, src, axis=0):
    return tgt.at[idx].add(src)
def _segment_sum(src, seg, n):
    return jax.ops.segment_sum(src, seg, n)
class _Rng:
    def __init__(self, key):
        self._k = key
    def _next(self):
        self._k, sub = jax.random.split(self._k)
        return sub
    def normal(self, shape):
        return jax.random.normal(self._next(), shape, dtype=jnp.bfloat16)
    def randint(self, lo, hi, shape):
        return jax.random.randint(self._next(), shape, lo, hi, dtype=jnp.int32)
    def uniform(self, shape, lo=0.0, hi=1.0):
        return jax.random.uniform(self._next(), shape, jnp.bfloat16, lo, hi)
    def permutation(self, n):
        return jax.random.permutation(self._next(), n)


kernel_name = 'gated_mix__ssm_conv_s5__geglu_ffn__prompt'

def setup_inputs():
    _rng = _Rng(jax.random.key(int.from_bytes(__import__("os").urandom(4), "little")))
    _w = (lambda a: (lambda t: t.astype(jnp.bfloat16) if jnp.issubdtype(t.dtype, jnp.floating) else t)(jnp.asarray(a)))
    def _A_setup():
        B, S, D = 1, 2048, 512
        P = D
        Lambda_re = -0.5 * jnp.exp((lambda *s: _rng.normal(s) * 0.4)(P))
        Lambda_im = (lambda *s: _rng.normal(s) * 0.4)(P) * 1.0
        B_re = (lambda *s: _rng.normal(s) * 0.4)(P, D) * (D ** -0.5)
        B_im = (lambda *s: _rng.normal(s) * 0.4)(P, D) * (D ** -0.5)
        C_re = (lambda *s: _rng.normal(s) * 0.4)(D, P) * (P ** -0.5)
        C_im = (lambda *s: _rng.normal(s) * 0.4)(D, P) * (P ** -0.5)
        log_dt = (lambda *s: _rng.normal(s) * 0.4)(P) * 0.3 - 2.0
        Dskip = (lambda *s: _rng.normal(s) * 0.4)(D)
        return {
            "x": _w((lambda *s: _rng.normal(s) * 0.05)(B, S, D)),
            "Lambda_re": _w(Lambda_re),
            "Lambda_im": _w(Lambda_im),
            "B_re": _w(B_re),
            "B_im": _w(B_im),
            "C_re": _w(C_re),
            "C_im": _w(C_im),
            "log_dt": _w(log_dt),
            "Dskip": _w(Dskip),
        }
    _A_in = _A_setup()

    def _B_setup():
        B, S, D, F = 1, 2048, 512, 1376
        return {
            "x": _w((lambda *s: _rng.normal(s) * 0.05)(B, S, D)),
            "w_gate": _w((lambda *s: _rng.normal(s) * 0.1)(D, F)),
            "w_up": _w((lambda *s: _rng.normal(s) * 0.1)(D, F)),
            "w_down": _w((lambda *s: _rng.normal(s) * 0.1)(F, D)),
        }
    _B_in = _B_setup()

    return {
        "A_x": _A_in["x"],
        "A_Lambda_re": _A_in["Lambda_re"],
        "A_Lambda_im": _A_in["Lambda_im"],
        "A_B_re": _A_in["B_re"],
        "A_B_im": _A_in["B_im"],
        "A_C_re": _A_in["C_re"],
        "A_C_im": _A_in["C_im"],
        "A_log_dt": _A_in["log_dt"],
        "A_Dskip": _A_in["Dskip"],
        "B_x": _B_in["x"],
        "B_w_gate": _B_in["w_gate"],
        "B_w_up": _B_in["w_up"],
        "B_w_down": _B_in["w_down"],
        "gate_w": _w((lambda *s: _rng.normal(s) * 0.05)(512) * 16.0),
    }

def reference(A_x, A_Lambda_re, A_Lambda_im, A_B_re, A_B_im, A_C_re, A_C_im, A_log_dt, A_Dskip, B_x, B_w_gate, B_w_up, B_w_down, gate_w):
    def _A_ref(x, Lambda_re, Lambda_im, B_re, B_im, C_re, C_im, log_dt, Dskip):
        Bsz, L, H = x.shape
        Lam = Lambda_re + 1j * Lambda_im
        Bmat = B_re + 1j * B_im
        Cmat = C_re + 1j * C_im
        dt = jnp.exp(log_dt)
        Lam_bar = jnp.exp(dt * Lam)
        B_bar = ((Lam_bar - 1.0) / Lam)[:, None] * Bmat
        Bu = jnp.einsum("bld,pd->blp", x + 0j, B_bar)
        h = jnp.zeros_like(Bu[:, 0, :])
        hs = []
        for t in range(L):
            h = Lam_bar[None, :] * h + Bu[:, t, :]
            hs.append(h)
        hseq = jnp.stack(hs, 1)
        y = 2.0 * jnp.einsum("blp,dp->bld", hseq, Cmat).real + x * Dskip[None, None, :]
        return y

    def _B_ref(x, w_gate, w_up, w_down):
        return (_gelu(x @ w_gate) * (x @ w_up)) @ w_down

    x = A_x
    g = _sigmoid((x * gate_w).sum(-1, keepdims=True))
    a = _A_ref(x, A_Lambda_re, A_Lambda_im, A_B_re, A_B_im, A_C_re, A_C_im, A_log_dt, A_Dskip)
    b = _B_ref(x, B_w_gate, B_w_up, B_w_down)
    return g * a + (1 - g) * b
```

```python
import numpy as np
import jax
import jax.numpy as jnp
from jax import lax
import jax.experimental.pallas as pl
import jax.experimental.pallas.tpu as pltpu

L = 2048
T = 128
NB = L // T
S = T // 8
Q = S + 1
Q2 = S // 2 + 1
RB = 8 * ((7 * Q + 2 * S + 7) // 8)
RH = 8 * ((7 * Q2 + S + 7) // 8)
XCH = [(0, 256), (256, 512), (512, 1024), (1024, 2048)]
NX = len(XCH)
CR = 16
PIN = 224
UNROLL = 8
P = 512
D = 512
F32 = jnp.float32
BF16 = jnp.bfloat16
NT = (((1,), (1,)), ((), ()))
C1 = float(np.sqrt(2.0 / np.pi))
C2 = float(np.sqrt(2.0 / np.pi) * 0.044715)


def _kernel(lre_hbm, lim_hbm, ldt_hbm, dsk_hbm, gw_hbm,
            x_hbm, bre_hbm, bim_hbm, cre_hbm, cim_hbm, wg_hbm, wu_hbm, wd_hbm, o_hbm,
            lre_ref, lim_ref, ldt_ref, dsk_ref, gw_ref,
            xs_ref, b_ref, c_ref, wg_ref, wu_ref, wd_ref, sems,
            par_ref, ct_ref, bu_ref, hw_ref, carry_ref, os_ref, osems):
    i = pl.program_id(0)

    def row(ref):
        return ref[...].astype(F32).reshape(1, -1)

    def weight_copy(n):
        src = (wg_hbm, wu_hbm, wd_hbm)[n]
        dst = (wg_ref, wu_ref, wd_ref)[n]
        return pltpu.make_async_copy(src, dst, sems.at[NX + 2 + n])

    @pl.when(i == 0)
    def _prologue():
        xcp = [pltpu.make_async_copy(x_hbm.at[pl.ds(r0, r1 - r0)], xs_ref.at[pl.ds(r0, r1 - r0)], sems.at[c])
               for c, (r0, r1) in enumerate(XCH)]
        cps = [
            pltpu.make_async_copy(cre_hbm, c_ref.at[0], sems.at[NX + 0]),
            pltpu.make_async_copy(cim_hbm, c_ref.at[1], sems.at[NX + 1]),
        ] + [weight_copy(n) for n in range(3)]
        bcp = [pltpu.make_async_copy(src.at[pl.ds(h * 256, 256)], b_ref.at[part, pl.ds(h * 256, 256)],
                                     sems.at[NX + 10 + 2 * part + h])
               for part, src in enumerate((bre_hbm, bim_hbm)) for h in range(2)]
        vcp = [pltpu.make_async_copy(a, b, sems.at[NX + 5 + n]) for n, (a, b) in enumerate(
            [(lre_hbm, lre_ref), (lim_hbm, lim_ref), (ldt_hbm, ldt_ref), (dsk_hbm, dsk_ref), (gw_hbm, gw_ref)])]
        for c in vcp:
            c.start()
        xcp[0].start()
        for c in bcp:
            c.start()
        for c in xcp[1:]:
            c.start()
        for c in cps:
            c.start()

        for c in vcp:
            c.wait()
        lr = row(lre_ref)
        li = row(lim_ref)
        dt = jnp.exp(row(ldt_ref)).astype(BF16).astype(F32)
        zr = dt * lr
        zi = dt * li
        r = lax.broadcasted_iota(jnp.int32, (8, P), 0)
        mult = jnp.where(r == 0, 1.0, jnp.where(r == 1, float(S), jnp.where(r == 2, 2.0 * S, 4.0 * S))).astype(F32)
        er = jnp.exp(mult * zr)
        ang = mult * zi
        pr = er * jnp.cos(ang)
        pi = er * jnp.sin(ang)
        par_ref[0] = pr
        par_ref[1] = pi
        lam_r = pr[0:1]
        lam_i = pi[0:1]
        den = lr * lr + li * li
        nr = lam_r - 1.0
        sr = 2.0 * (nr * lr + lam_i * li) / den
        si = 2.0 * (lam_i * lr - nr * li) / den
        carry_ref[...] = jnp.zeros_like(carry_ref)
        nsi = -si
        never = i > 0

        tail = []

        def pin(spare_ref):
            spare_ref[0:16, 0:128] = tail[-1].astype(BF16)

        for c, (r0, r1) in enumerate(XCH):
            if c > 0:
                pin(xs_ref.at[pl.ds(L, 16)])
            xcp[c].wait()
            x = xs_ref[r0:r1, :]
            for part, n0, n1 in ([(p, h * 256, h * 256 + 256) for p in range(2) for h in range(2)] if c == 0
                                 else [(0, 0, P), (1, 0, P)]):
                if c == 0:
                    if part + n0 > 0:
                        pin(b_ref.at[2])
                    bcp[2 * part + n0 // 256].wait()
                if c == NX - 1 and part == 1:
                    pin(c_ref.at[2])
                    cps[0].wait()
                    cps[1].wait()
                bu = lax.dot_general(x, b_ref[part, n0:n1, :], NT, preferred_element_type=F32)
                tail.append(bu[r1 - r0 - PIN:r1 - r0 - PIN + 16, n1 - n0 - 128:n1 - n0])
                if c == NX - 1 and part == 1:
                    for r in range(0, D, CR):
                        for k in range(4):
                            ls = slice(k * 128, (k + 1) * 128)
                            q = (r // CR) * 4 + k
                            p0 = 8 * ((q * ((r1 - r0) // 8 - 2)) // (4 * D // CR))
                            cr = jnp.where(never, bu[p0:p0 + CR, 0:128], c_ref[0, r:r + CR, ls].astype(F32))
                            ci = c_ref[1, r:r + CR, ls].astype(F32)
                            ct_ref[r:r + CR, k * 128:(k + 1) * 128] = (cr * sr[:, ls] - ci * si[:, ls]).astype(BF16)
                            ct_ref[r:r + CR, P + k * 128:P + (k + 1) * 128] = (cr * nsi[:, ls] - ci * sr[:, ls]).astype(BF16)
                for k in range(n0 // 128, n1 // 128):
                    for m in range((r1 - r0) // 8):
                        t = r0 + 8 * m
                        blk, tt = t // T, t % T
                        sc, j0 = tt // S, tt % S
                        bu_ref[blk, 4 * part + k, pl.ds(Q * sc + 2 * j0, 8, stride=2), :] = (
                            bu[8 * m:8 * m + 8, k * 128 - n0:(k + 1) * 128 - n0])

    def out_copy(blk):
        r0 = pl.multiple_of(blk * T, T)
        return pltpu.make_async_copy(os_ref.at[pl.ds(r0, T)], o_hbm.at[pl.ds(r0, T)], osems.at[blk])

    def main(blk, prev):
        r0 = pl.multiple_of(blk * T, T)
        x = xs_ref[pl.ds(r0, T), :]
        sub = lax.broadcasted_iota(jnp.int32, (8, 128), 0)
        last = {}
        never = blk < 0

        def scan(k):
            ls = slice(k * 128, (k + 1) * 128)
            pw_r = par_ref[0, :, ls]
            pw_i = par_ref[1, :, ls]
            lr = jnp.broadcast_to(pw_r[0:1], (8, 128))
            li = jnp.broadcast_to(pw_i[0:1], (8, 128))

            def ld(j, k=k):
                return (bu_ref[blk, k, pl.ds(2 * j, 8, stride=Q), :],
                        bu_ref[blk, 4 + k, pl.ds(2 * j, 8, stride=Q), :])
            s_r, s_i = ld(0)
            dep = last[k - 1] if k > 0 else prev.get('h')
            if dep is not None:
                s_r = jnp.where(never, dep, s_r)
            for j in range(1, S):
                ur, ui = ld(j)
                s_r, s_i = lr * s_r - li * s_i + ur, lr * s_i + li * s_r + ui
            er_prev = carry_ref[0, k]
            ei_prev = carry_ref[1, k]
            vr = jnp.where(sub == 0, pltpu.roll(er_prev, 1, 0), pltpu.roll(s_r, 1, 0))
            vi = jnp.where(sub == 0, pltpu.roll(ei_prev, 1, 0), pltpu.roll(s_i, 1, 0))
            for n, d in enumerate((1, 2, 4)):
                mr = jnp.broadcast_to(pw_r[n + 1:n + 2], (8, 128))
                mi = jnp.broadcast_to(pw_i[n + 1:n + 2], (8, 128))
                tr = jnp.where(sub >= d, pltpu.roll(vr, d, 0), 0.0)
                ti = jnp.where(sub >= d, pltpu.roll(vi, d, 0), 0.0)
                vr, vi = vr + (mr * tr - mi * ti), vi + (mr * ti + mi * tr)
            mr = jnp.broadcast_to(pw_r[1:2], (8, 128))
            mi = jnp.broadcast_to(pw_i[1:2], (8, 128))
            carry_ref[0, k] = mr * vr - mi * vi + s_r
            carry_ref[1, k] = mr * vi + mi * vr + s_i
            hr, hi = vr, vi
            for m in range(S // 2):
                ur, ui = ld(2 * m)
                ar, ai = lr * hr - li * hi + ur, lr * hi + li * hr + ui
                ur, ui = ld(2 * m + 1)
                hr, hi = lr * ar - li * ai + ur, lr * ai + li * ar + ui
                hw_ref[k, pl.ds(2 * m, 8, stride=Q2), :] = pltpu.pack_elementwise([ar, hr], packed_dtype=BF16)
                hw_ref[4 + k, pl.ds(2 * m, 8, stride=Q2), :] = pltpu.pack_elementwise([ai, hi], packed_dtype=BF16)
            last[k] = hr

        for k in range(4):
            scan(k)
        prev['h'] = last[3]

        gt = lax.dot_general(x, wg_ref[...], NT, preferred_element_type=F32)
        up = lax.dot_general(x, wu_ref[...], NT, preferred_element_type=F32)
        th = jnp.tanh(gt * (C1 + C2 * (gt * gt)))
        gu = gt * up
        act = (gu * th + gu).astype(BF16)

        cols = []
        for k in range(8):
            parts = []
            for m in range(T // 16):
                c, m0 = (8 * m) // (S // 2), (8 * m) % (S // 2)
                parts.append(hw_ref[k, pl.ds(Q2 * c + 2 * m0, 8, stride=2), :])
            cols.append(pltpu.bitcast(jnp.concatenate(parts, axis=0), BF16))
        h = jnp.concatenate(cols, axis=1)
        ya = lax.dot_general(h, ct_ref[...], NT, preferred_element_type=F32)
        yb = jnp.dot(act, wd_ref[...], preferred_element_type=F32)

        xf = x.astype(F32)
        g = jax.nn.sigmoid(jnp.sum(xf * row(gw_ref), axis=-1, keepdims=True))
        a = ya + xf * row(dsk_ref)
        os_ref[pl.ds(r0, T), :] = g * a + (0.5 - 0.5 * g) * yb
        out_copy(blk).start()

    @pl.when(i > 0)
    def _main():
        for n in range(3):
            weight_copy(n).wait()

        @pl.loop(0, NB // UNROLL)
        def _(it):
            prev = {}
            for u in range(UNROLL):
                main(it * UNROLL + u, prev)
        for blk in range(NB):
            out_copy(blk).wait()


@jax.jit
def pallas_gated_mix__ssm_conv_s5__geglu_ffn__prompt_kernel(
    A_x, A_Lambda_re, A_Lambda_im, A_B_re, A_B_im, A_C_re, A_C_im, A_log_dt, A_Dskip,
    B_x, B_w_gate, B_w_up, B_w_down, gate_w,
):
    del B_x
    Bn = A_x.shape[0]
    Ff = B_w_gate.shape[1]
    assert A_x.shape == (1, L, D) and A_B_re.shape == (P, D)
    x2 = A_x.reshape(L, D)
    hbm = pl.BlockSpec(memory_space=pltpu.HBM)
    out = pl.pallas_call(
        _kernel,
        grid=(2,),
        in_specs=[hbm] * 13,
        out_specs=hbm,
        out_shape=jax.ShapeDtypeStruct((L, D), F32),
        scratch_shapes=[
            *[pltpu.VMEM((D,), BF16)] * 5,
            pltpu.VMEM((L + 16, D), BF16),
            pltpu.VMEM((3, P, D), BF16),
            pltpu.VMEM((3, D, P), BF16),
            pltpu.VMEM((Ff, D), BF16),
            pltpu.VMEM((Ff, D), BF16),
            pltpu.VMEM((Ff, D), BF16),
            pltpu.SemaphoreType.DMA((NX + 14,)),
            pltpu.VMEM((2, 8, P), F32),
            pltpu.VMEM((D, 2 * P), BF16),
            pltpu.VMEM((NB, 8, RB, 128), F32),
            pltpu.VMEM((8, RH, 128), jnp.uint32),
            pltpu.VMEM((2, 4, 8, 128), F32),
            pltpu.VMEM((L, D), F32),
            pltpu.SemaphoreType.DMA((NB,)),
        ],
        compiler_params=pltpu.CompilerParams(
            dimension_semantics=("arbitrary",), vmem_limit_bytes=100 * 1024 * 1024,
            flags={"XLA_TPU_RESCHEDULE_DMA_DONES": True}),
    )(A_Lambda_re, A_Lambda_im, A_log_dt, A_Dskip, gate_w,
      x2, A_B_re, A_B_im, A_C_re, A_C_im, B_w_gate.T, B_w_up.T, B_w_down)
    return out.reshape(Bn, L, D)
```
